```python
import os as _os
_os.environ.setdefault("JAX_PLATFORMS", "cpu")
import jax
import jax.numpy as jnp

def _softmax(x, axis=-1):
    return jax.nn.softmax(x, axis=axis)
def _gelu(x):
    return jax.nn.gelu(x, approximate=True)
def _silu(x):
    return jax.nn.silu(x)
def _sigmoid(x):
    return jax.nn.sigmoid(x)
def _layernorm(x, axis=-1, eps=1e-5):
    m = jnp.mean(x, axis=axis, keepdims=True)
    v = jnp.var(x, axis=axis, keepdims=True)
    return (x - m) / jnp.sqrt(v + eps)
def _scatter_add(tgt, idx, src, axis=0):
    return tgt.at[idx].add(src)
def _segment_sum(src, seg, n):
    return jax.ops.segment_sum(src, seg, n)
class _Rng:
    def __init__(self, key):
        self._k = key
    def _next(self):
        self._k, sub = jax.random.split(self._k)
        return sub
    def normal(self, shape):
        return jax.random.normal(self._next(), shape, dtype=jnp.bfloat16)
    def randint(self, lo, hi, shape):
        return jax.random.randint(self._next(), shape, lo, hi, dtype=jnp.int32)
    def uniform(self, shape, lo=0.0, hi=1.0):
        return jax.random.uniform(self._next(), shape, jnp.bfloat16, lo, hi)
    def permutation(self, n):
        return jax.random.permutation(self._next(), n)


kernel_name = 'standalone__detection_seg_fpn_lateral__vision'

def setup_inputs():
    _rng = _Rng(jax.random.key(int.from_bytes(__import__("os").urandom(4), "little")))
    _w = (lambda a: (lambda t: t.astype(jnp.bfloat16) if jnp.issubdtype(t.dtype, jnp.floating) else t)(jnp.asarray(a)))
    H = W = (256 // 2) * 2
    C = 384
    k = 1
    return {
        "c_fine": _w((lambda *s: _rng.normal(s) * 0.05)(1, H, W, C)),
        "p_coarse": _w((lambda *s: _rng.normal(s) * 0.05)(1, H // 2, W // 2, C)),
        "w_lat": _w((lambda *s: _rng.normal(s) * 0.05)(C, C)),
        "w_out": _w((lambda *s: _rng.normal(s) * 0.05)(k, k, C, C)),
    }

def reference(c_fine, p_coarse, w_lat, w_out):
    B, H, W, C = c_fine.shape
    k = 1
    lat = jnp.einsum("bhwc,cd->bhwd", c_fine, w_lat)
    up = jnp.repeat(jnp.repeat(p_coarse, 2, axis=1), 2, axis=2)
    m = lat + up
    pad = k // 2
    mp = jnp.pad(m, ((0, 0), (pad, pad), (pad, pad), (0, 0)))
    o = None
    for di in range(k):
        for dj in range(k):
            t = jnp.einsum("bhwc,cd->bhwd", mp[:, di:di + H, dj:dj + W, :], w_out[di, dj])
            o = t if o is None else o + t
    return o
```

```python
import jax
import jax.numpy as jnp
import jax.experimental.pallas as pl
import jax.experimental.pallas.tpu as pltpu


def _up2(q):
    w = pltpu.pack_elementwise([q, q], packed_dtype=jnp.bfloat16)
    return pltpu.bitcast(w, jnp.bfloat16).astype(jnp.float32)


@jax.jit
def pallas_standalone__detection_seg_fpn_lateral__vision_kernel(
    c_fine: jax.Array,
    p_coarse: jax.Array,
    w_lat: jax.Array,
    w_out: jax.Array,
):
    B, H, W, C = c_fine.shape
    R = 4

    def kernel_function(c_ref, p_ref, wl_ref, wo_ref, o_ref, wc_ref):
        wo = wo_ref[...]

        @pl.when(pl.program_id(0) == 0)
        def _():
            wc_ref[...] = jnp.dot(
                wl_ref[...], wo, preferred_element_type=jnp.float32
            ).astype(wc_ref.dtype)

        wc = wc_ref[...]
        for r in range(R):
            u = _up2(jnp.dot(p_ref[r], wo, preferred_element_type=jnp.float32))
            for j in range(2):
                acc = jnp.dot(c_ref[2 * r + j], wc, preferred_element_type=jnp.float32)
                o_ref[2 * r + j] = (acc + u).astype(o_ref.dtype)

    out = pl.pallas_call(
        kernel_function,
        grid=(B * H // 2 // R,),
        in_specs=[
            pl.BlockSpec((2 * R, W, C), lambda i: (i, 0, 0)),
            pl.BlockSpec((R, W // 2, C), lambda i: (i, 0, 0)),
            pl.BlockSpec((C, C), lambda i: (0, 0)),
            pl.BlockSpec((C, C), lambda i: (0, 0)),
        ],
        out_specs=pl.BlockSpec((2 * R, W, C), lambda i: (i, 0, 0)),
        out_shape=jax.ShapeDtypeStruct((B * H, W, C), c_fine.dtype),
        scratch_shapes=[pltpu.VMEM((C, C), jnp.bfloat16)],
        compiler_params=pltpu.CompilerParams(
            dimension_semantics=("arbitrary",), vmem_limit_bytes=64 << 20
        ),
    )(
        c_fine.reshape(B * H, W, C),
        p_coarse.reshape(B * H // 2, W // 2, C),
        w_lat,
        w_out.reshape(C, C),
    )
    return out.reshape(B, H, W, C)
```

```python
import jax
import jax.numpy as jnp
import jax.experimental.pallas as pl
import jax.experimental.pallas.tpu as pltpu

_STREAMS = 16
_COLS = 32
_WRITE_PIXELS = 32
_WRITE_QUEUES = 2
_WRITE_BACKLOG = 8


def _dot(a, b):
    return jnp.dot(a, b, preferred_element_type=jnp.float32)


def _repeat_rows_twice(x):
    x = x.astype(jnp.bfloat16).astype(jnp.float32)
    bits = jax.lax.bitcast_convert_type(x, jnp.uint32)
    return pltpu.bitcast(bits | (bits >> 16), jnp.bfloat16).astype(jnp.float32)


def _fpn_kernel(
    c_hbm, p_hbm, w_lat_hbm, w_out_hbm, o_hbm,
    c_vmem, p_vmem, o_vmem, w_lat_vmem, w_out_vmem, w_fused_vmem, write_sem,
):
    streams, rows, cols, chans = p_hbm.shape
    col_blocks = cols // _COLS
    steps = rows * col_blocks
    first_write_step = steps * 9 // 16
    backlog = min(_WRITE_BACKLOG, first_write_step)
    per_queue = streams // _WRITE_QUEUES

    def coarse_row(step):
        return step // col_blocks

    def coarse_cols(step):
        return pl.ds(pl.multiple_of(step % col_blocks * _COLS, _COLS), _COLS)

    def fine_cols(step, offset=0, size=2 * _COLS):
        start = step % col_blocks * (2 * _COLS) + offset
        return pl.ds(pl.multiple_of(start, size), size)

    def start_write(step):
        for dy in range(2):
            for offset in range(0, 2 * _COLS, _WRITE_PIXELS):
                for queue in range(_WRITE_QUEUES):
                    idx = (
                        pl.ds(queue * per_queue, per_queue),
                        2 * coarse_row(step) + dy,
                        fine_cols(step, offset, _WRITE_PIXELS),
                    )
                    pltpu.make_async_copy(
                        o_vmem.at[idx], o_hbm.at[idx], write_sem
                    ).start(priority=queue)

    def writes_started(computed):
        started = jnp.minimum(computed, backlog + 2 * (computed - first_write_step))
        return jnp.where(computed == steps, steps, started)

    def compute(step):
        row = coarse_row(step)
        p = p_vmem[:, row, coarse_cols(step), :].reshape(-1, chans)
        top_down = _repeat_rows_twice(_dot(p, w_out_vmem[...]))
        for dy in range(2):
            idx = (slice(None), 2 * row + dy, fine_cols(step), slice(None))
            out = _dot(c_vmem[idx].reshape(-1, chans), w_fused_vmem[...]) + top_down
            o_vmem[idx] = out.astype(o_vmem.dtype).reshape(streams, 2 * _COLS, chans)

    def run(c_sems, p_sems, w_sems):
        def c_read(step):
            idx = (slice(None), pl.ds(2 * coarse_row(step), 2), fine_cols(step))
            return pltpu.make_async_copy(c_hbm.at[idx], c_vmem.at[idx], c_sems.at[step])

        def p_read(step):
            idx = (slice(None), coarse_row(step), coarse_cols(step))
            return pltpu.make_async_copy(p_hbm.at[idx], p_vmem.at[idx], p_sems.at[step])

        def wait_reads(step):
            c_read(step).wait()
            p_read(step).wait()

        w_lat_read = pltpu.async_copy(w_lat_hbm, w_lat_vmem, w_sems.at[0])
        w_out_read = pltpu.async_copy(w_out_hbm, w_out_vmem, w_sems.at[1])

        @pl.loop(0, steps)
        def _(step):
            c_read(step).start()
            p_read(step).start()

        w_lat_read.wait()
        w_out_read.wait()
        w_fused = _dot(w_lat_vmem[...], w_out_vmem[...])
        w_fused_vmem[...] = w_fused.astype(w_fused_vmem.dtype)

        @pl.loop(0, steps)
        def _(step):
            @pl.when(step < first_write_step)
            def _():
                wait_reads(step)

            @pl.when(step == first_write_step)
            def _():
                last = step + (steps - 1 - first_write_step)
                pl.loop(first_write_step, steps - 1)(wait_reads)
                c_read(last).wait()
                pl.loop(0, backlog)(start_write)
                p_read(last).wait()

            compute(step)

            @pl.when(step >= first_write_step)
            def _():
                pl.loop(writes_started(step), writes_started(step + 1))(start_write)

    pl.run_scoped(
        run,
        pltpu.SemaphoreType.DMA((steps,)),
        pltpu.SemaphoreType.DMA((steps,)),
        pltpu.SemaphoreType.DMA((2,)),
    )
    pltpu.make_async_copy(o_vmem, o_hbm, write_sem).wait()


@jax.jit
def pallas_standalone__detection_seg_fpn_lateral__vision_kernel(
    c_fine: jax.Array,
    p_coarse: jax.Array,
    w_lat: jax.Array,
    w_out: jax.Array,
):
    B, H, W, C = c_fine.shape
    assert p_coarse.shape == (B, H // 2, W // 2, C) and w_out.shape == (1, 1, C, C)
    assert H % 2 == 0 and (B * H) % (2 * _STREAMS) == 0 and W % (2 * _COLS) == 0
    fine = (_STREAMS, B * H // _STREAMS, W, C)
    coarse = (_STREAMS, B * H // (2 * _STREAMS), W // 2, C)

    out = pl.pallas_call(
        _fpn_kernel,
        in_specs=[pl.BlockSpec(memory_space=pl.ANY)] * 4,
        out_specs=pl.BlockSpec(memory_space=pl.ANY),
        out_shape=jax.ShapeDtypeStruct(fine, c_fine.dtype),
        scratch_shapes=[
            pltpu.VMEM(fine, c_fine.dtype),
            pltpu.VMEM(coarse, p_coarse.dtype),
            pltpu.VMEM(fine, c_fine.dtype),
            pltpu.VMEM((C, C), w_lat.dtype),
            pltpu.VMEM((C, C), w_out.dtype),
            pltpu.VMEM((C, C), c_fine.dtype),
            pltpu.SemaphoreType.DMA(()),
        ],
        compiler_params=pltpu.CompilerParams(vmem_limit_bytes=120 * 1024 * 1024),
    )(c_fine.reshape(fine), p_coarse.reshape(coarse), w_lat, w_out.reshape(C, C))
    return out.reshape(B, H, W, C)
```

```python
import jax
import jax.numpy as jnp
import jax.experimental.pallas as pl
import jax.experimental.pallas.tpu as pltpu

_STREAMS = 16
_COLS = 32
_WRITE_PIXELS = 32
_WRITE_QUEUES = 2
_WRITE_BACKLOG = 8


def _dot(a, b):
    return jnp.dot(a, b, preferred_element_type=jnp.float32)


def _repeat_rows_twice(x):
    x = x.astype(jnp.bfloat16).astype(jnp.float32)
    bits = jax.lax.bitcast_convert_type(x, jnp.uint32)
    return pltpu.bitcast(bits | (bits >> 16), jnp.bfloat16).astype(jnp.float32)


def _fpn_kernel(
    c_hbm, p_hbm, w_lat_hbm, w_out_hbm, o_hbm,
    c_vmem, p_vmem, o_vmem, w_lat_vmem, w_out_vmem, w_fused_vmem, write_sem,
):
    streams, rows, cols, chans = p_hbm.shape
    col_blocks = cols // _COLS
    steps = rows * col_blocks
    first_write_step = steps * 3 // 5
    backlog = min(_WRITE_BACKLOG, first_write_step)
    per_queue = streams // _WRITE_QUEUES

    def coarse_row(step):
        return step // col_blocks

    def coarse_cols(step):
        return pl.ds(pl.multiple_of(step % col_blocks * _COLS, _COLS), _COLS)

    def fine_cols(step, offset=0, size=2 * _COLS):
        start = step % col_blocks * (2 * _COLS) + offset
        return pl.ds(pl.multiple_of(start, size), size)

    def start_write(unit):
        for offset in range(0, 2 * _COLS, _WRITE_PIXELS):
            for queue in range(_WRITE_QUEUES):
                idx = (
                    pl.ds(queue * per_queue, per_queue),
                    unit // col_blocks,
                    fine_cols(unit, offset, _WRITE_PIXELS),
                )
                pltpu.make_async_copy(
                    o_vmem.at[idx], o_hbm.at[idx], write_sem
                ).start(priority=queue)

    def writes_started(computed):
        ready = computed // col_blocks * (2 * col_blocks) + computed % col_blocks
        paced = jnp.minimum(ready, backlog + 4 * (computed - first_write_step))
        return jnp.where(computed == steps, ready, paced)

    def compute(step):
        row = coarse_row(step)
        p = p_vmem[:, row, coarse_cols(step), :].reshape(-1, chans)
        top_down = _repeat_rows_twice(_dot(p, w_out_vmem[...]))
        for dy in range(2):
            idx = (slice(None), 2 * row + dy, fine_cols(step), slice(None))
            out = _dot(c_vmem[idx].reshape(-1, chans), w_fused_vmem[...]) + top_down
            o_vmem[idx] = out.astype(o_vmem.dtype).reshape(streams, 2 * _COLS, chans)

    def run(c_sems, p_sems, w_sems):
        def c_read(step):
            idx = (slice(None), pl.ds(2 * coarse_row(step), 2), fine_cols(step))
            return pltpu.make_async_copy(c_hbm.at[idx], c_vmem.at[idx], c_sems.at[step])

        def p_read(step):
            idx = (slice(None), coarse_row(step), coarse_cols(step))
            return pltpu.make_async_copy(p_hbm.at[idx], p_vmem.at[idx], p_sems.at[step])

        def wait_reads(step):
            c_read(step).wait()
            p_read(step).wait()

        w_lat_read = pltpu.async_copy(w_lat_hbm, w_lat_vmem, w_sems.at[0])
        w_out_read = pltpu.async_copy(w_out_hbm, w_out_vmem, w_sems.at[1])

        @pl.loop(0, steps)
        def _(step):
            c_read(step).start()
            p_read(step).start()

        w_lat_read.wait()
        w_out_read.wait()
        w_fused = _dot(w_lat_vmem[...], w_out_vmem[...])
        w_fused_vmem[...] = w_fused.astype(w_fused_vmem.dtype)

        @pl.loop(0, steps)
        def _(step):
            @pl.when(step < first_write_step)
            def _():
                wait_reads(step)

            @pl.when(step == first_write_step)
            def _():
                last = step + (steps - 1 - first_write_step)
                pl.loop(first_write_step, steps - 1)(wait_reads)
                c_read(last).wait()
                pl.loop(0, backlog)(start_write)
                p_read(last).wait()

            compute(step)

            @pl.when(step >= first_write_step)
            def _():
                pl.loop(writes_started(step), writes_started(step + 1))(start_write)

    pl.run_scoped(
        run,
        pltpu.SemaphoreType.DMA((steps,)),
        pltpu.SemaphoreType.DMA((steps,)),
        pltpu.SemaphoreType.DMA((2,)),
    )
    pltpu.make_async_copy(o_vmem, o_hbm, write_sem).wait()


@jax.jit
def pallas_standalone__detection_seg_fpn_lateral__vision_kernel(
    c_fine: jax.Array,
    p_coarse: jax.Array,
    w_lat: jax.Array,
    w_out: jax.Array,
):
    B, H, W, C = c_fine.shape
    assert p_coarse.shape == (B, H // 2, W // 2, C) and w_out.shape == (1, 1, C, C)
    assert H % 2 == 0 and (B * H) % (2 * _STREAMS) == 0 and W % (2 * _COLS) == 0
    fine = (_STREAMS, B * H // _STREAMS, W, C)
    coarse = (_STREAMS, B * H // (2 * _STREAMS), W // 2, C)

    out = pl.pallas_call(
        _fpn_kernel,
        in_specs=[pl.BlockSpec(memory_space=pl.ANY)] * 4,
        out_specs=pl.BlockSpec(memory_space=pl.ANY),
        out_shape=jax.ShapeDtypeStruct(fine, c_fine.dtype),
        scratch_shapes=[
            pltpu.VMEM(fine, c_fine.dtype),
            pltpu.VMEM(coarse, p_coarse.dtype),
            pltpu.VMEM(fine, c_fine.dtype),
            pltpu.VMEM((C, C), w_lat.dtype),
            pltpu.VMEM((C, C), w_out.dtype),
            pltpu.VMEM((C, C), c_fine.dtype),
            pltpu.SemaphoreType.DMA(()),
        ],
        compiler_params=pltpu.CompilerParams(vmem_limit_bytes=120 * 1024 * 1024),
    )(c_fine.reshape(fine), p_coarse.reshape(coarse), w_lat, w_out.reshape(C, C))
    return out.reshape(B, H, W, C)
```
